```python
import jax
import jax.numpy as jnp

def _softmax(x, axis=-1):
    return jax.nn.softmax(x, axis=axis)
def _gelu(x):
    return jax.nn.gelu(x, approximate=True)
def _silu(x):
    return jax.nn.silu(x)
def _sigmoid(x):
    return jax.nn.sigmoid(x)
def _layernorm(x, axis=-1, eps=1e-5):
    m = jnp.mean(x, axis=axis, keepdims=True)
    v = jnp.var(x, axis=axis, keepdims=True)
    return (x - m) / jnp.sqrt(v + eps)
def _scatter_add(tgt, idx, src, axis=0):
    return tgt.at[idx].add(src)
def _segment_sum(src, seg, n):
    return jax.ops.segment_sum(src, seg, n)
class _Rng:
    def __init__(self, key):
        self._k = key
    def _next(self):
        self._k, sub = jax.random.split(self._k)
        return sub
    def normal(self, shape):
        return jax.random.normal(self._next(), shape, dtype=jnp.bfloat16)
    def randint(self, lo, hi, shape):
        return jax.random.randint(self._next(), shape, lo, hi, dtype=jnp.int32)
    def uniform(self, shape, lo=0.0, hi=1.0):
        return jax.random.uniform(self._next(), shape, jnp.bfloat16, lo, hi)
    def permutation(self, n):
        return jax.random.permutation(self._next(), n)


kernel_name = 'gated_mix__compressed_kv_cla__gqa_block_cached__decode'

def setup_inputs():
    _rng = _Rng(jax.random.key(int.from_bytes(__import__("os").urandom(4), "little")))
    _w = (lambda a: (lambda t: t.astype(jnp.bfloat16) if jnp.issubdtype(t.dtype, jnp.floating) else t)(jnp.asarray(a)))
    def _A_setup():
        B, H, Sq, Sk, D, M = 1, 32, 1, 4096, 128, 640
        Dc = 4 * D
        return {
            "x": _w((lambda *s: _rng.normal(s) * 0.05)(B, Sq, M)),
            "c_kv": _w((lambda *s: _rng.normal(s) * 0.05)(B, Sk, Dc)),
            "w_q": _w((lambda *s: _rng.normal(s) * 0.05)(M, H, D) * (M ** -0.5)),
            "w_uk": _w((lambda *s: _rng.normal(s) * 0.05)(Dc, H, D) * (Dc ** -0.5)),
            "w_uv": _w((lambda *s: _rng.normal(s) * 0.05)(Dc, H, D) * (Dc ** -0.5)),
            "w_o": _w((lambda *s: _rng.normal(s) * 0.05)(H, D, M) * ((H * D) ** -0.5)),
        }
    _A_in = _A_setup()

    def _B_setup():
        B, Sq, D = 1, 1, 640
        Hq, Hkv, Sk, Dh = 32, 32, 4096, 128
        assert Hq % Hkv == 0, (Hq, Hkv)
        return {
            "x": _w((lambda *s: _rng.normal(s) * 0.05)(B, Sq, D)),
            "k_cache": _w((lambda *s: _rng.normal(s) * 0.05)(B, Hkv, Sk, Dh)),
            "v_cache": _w((lambda *s: _rng.normal(s) * 0.05)(B, Hkv, Sk, Dh)),
            "wq": _w((lambda *s: _rng.normal(s) * 0.05)(D, Hq * Dh) * (D ** -0.5)),
            "wo": _w((lambda *s: _rng.normal(s) * 0.05)(Hq * Dh, D) * ((Hq * Dh) ** -0.5)),
        }
    _B_in = _B_setup()

    return {
        "A_x": _A_in["x"],
        "A_c_kv": _A_in["c_kv"],
        "A_w_q": _A_in["w_q"],
        "A_w_uk": _A_in["w_uk"],
        "A_w_uv": _A_in["w_uv"],
        "A_w_o": _A_in["w_o"],
        "B_x": _B_in["x"],
        "B_k_cache": _B_in["k_cache"],
        "B_v_cache": _B_in["v_cache"],
        "B_wq": _B_in["wq"],
        "B_wo": _B_in["wo"],
        "gate_w": _w((lambda *s: _rng.normal(s) * 0.05)(640)),
    }

def reference(A_x, A_c_kv, A_w_q, A_w_uk, A_w_uv, A_w_o, B_x, B_k_cache, B_v_cache, B_wq, B_wo, gate_w):
    def _A_ref(x, c_kv, w_q, w_uk, w_uv, w_o):
        B, Sq, M = x.shape[0], x.shape[1], x.shape[2]
        Sk = c_kv.shape[1]
        H, D = w_q.shape[1], w_q.shape[2]
        q = jnp.einsum("bqm,mhd->bhqd", x, w_q)
        k = jnp.einsum("bkc,chd->bhkd", c_kv, w_uk)
        v = jnp.einsum("bkc,chd->bhkd", c_kv, w_uv)
        scores = jnp.einsum("bhqd,bhkd->bhqk", q, k) * (D ** -0.5)
        off = Sk - Sq
        qi = jnp.arange(Sq)[:, None]
        kj = jnp.arange(Sk)[None, :]
        cmask = kj <= (qi + off)
        scores = jnp.where(cmask[None, None], scores, -1e9)
        p = _softmax(scores, axis=-1)
        ctx = jnp.einsum("bhqk,bhkd->bhqd", p, v)
        return jnp.einsum("bhqd,hdm->bqm", ctx, w_o)

    def _B_ref(x, k_cache, v_cache, wq, wo):
        B, Sq, D = x.shape
        Hq, Dh = 32, 128
        Hkv = k_cache.shape[1]
        rep = Hq // Hkv
        q = (lambda x, *d: x.transpose(*d))((x @ wq).reshape(B, Sq, Hq, Dh), 0, 2, 1, 3)
        k = jnp.repeat(k_cache, rep, axis=1)
        v = jnp.repeat(v_cache, rep, axis=1)
        scores = jnp.einsum("bhqd,bhkd->bhqk", q, k) * (Dh ** -0.5)
        p = _softmax(scores, axis=-1)
        o = jnp.einsum("bhqk,bhkd->bhqd", p, v)
        return (lambda x, *d: x.transpose(*d))(o, 0, 2, 1, 3).reshape(B, Sq, Hq * Dh) @ wo

    x = A_x
    g = _sigmoid((x * gate_w).sum(-1, keepdims=True))
    a = _A_ref(x, A_c_kv, A_w_q, A_w_uk, A_w_uv, A_w_o)
    b = _B_ref(x, B_k_cache, B_v_cache, B_wq, B_wo)
    return g * a + (1 - g) * b
```

```python
import functools
import numpy as np
import jax
import jax.numpy as jnp
from jax import lax
from jax.experimental import pallas as pl
from jax.experimental.pallas import tpu as pltpu

H, DH, M, DC, S = 32, 128, 640, 512, 4096
F32, BF16 = jnp.float32, jnp.bfloat16
NT = (((1,), (1,)), ((), ()))


def _splits(rows, n, align=16):
    u = rows // align
    base, rem = divmod(u, n)
    sizes = [(base + (1 if i < rem else 0)) * align for i in range(n)]
    offs = np.cumsum([0] + sizes[:-1]).tolist()
    return list(zip(offs, sizes))


def _make(D=2, nsub_kv=24, sub_bytes=44 * 1024, two_q=True, compute=True, LA=64):
    NBUF = D + 1

    def kernel(x_hbm, ckv_hbm, awq_hbm, wuk_hbm, wuv_hbm, awo_hbm, k_hbm, v_hbm,
               bwq_hbm, bwo_hbm, gate_hbm,
               out_ref,
               x_v, gate_v, ckv_v, awq_v, wuk_v, wuv_v, awo_v, bwq_v, bwo_v, k_v, v_v,
               qb_s, sem_w, sem_kv):
        def pieces(rows, cols):
            unit = 16 * cols * 2
            half = rows // 2
            out = []
            if unit <= sub_bytes:
                for (o, r) in _splits(half, max(1, int(np.ceil(half * cols * 2 / sub_bytes)))):
                    out.append((o, r, 0, cols))
            else:
                ncol = int(np.ceil(unit / sub_bytes))
                for o in range(0, half, 16):
                    for (co, cw) in _splits(cols, ncol, 128):
                        out.append((o, 16, co, cw))
            return half, out

        stream = []
        item_end = []
        issued = [0]

        def add_item(src, dst, sem):
            rows, cols = dst.shape
            half, ps = pieces(rows, cols)
            for (o, r, co, cw) in ps:
                for q in range(2):
                    ro = o + q * half
                    def th(ro=ro, r=r, co=co, cw=cw, q=q):
                        pltpu.make_async_copy(src.at[pl.ds(ro, r), pl.ds(co, cw)], dst.at[pl.ds(ro, r), pl.ds(co, cw)], sem).start(priority=q if two_q else 0)
                    stream.append(th)
            item_end.append(len(stream))

        def add_kv_static(h, slot):
            for (o, r) in kv_sp:
                def thk(o=o, r=r):
                    pltpu.make_async_copy(k_hbm.at[h, pl.ds(o, r)], k_v.at[slot, pl.ds(o, r)], sem_kv.at[0, slot]).start(priority=0)
                def thv(o=o, r=r):
                    pltpu.make_async_copy(v_hbm.at[h, pl.ds(o, r)], v_v.at[slot, pl.ds(o, r)], sem_kv.at[1, slot]).start(priority=1 if two_q else 0)
                stream.append(thk); stream.append(thv)

        def issue_until(n):
            n = min(n, len(stream))
            while issued[0] < n:
                stream[issued[0]]()
                issued[0] += 1

        def need(i):
            issue_until(item_end[i] + LA)
            wait_item(items[i][1], sem_w.at[i])

        def wait_item(dst, sem):
            pltpu.make_async_copy(dst, dst, sem).wait()

        kv_sp = _splits(S, nsub_kv)

        def start_kv(h, slot):
            for (o, r) in kv_sp:
                pltpu.make_async_copy(k_hbm.at[h, pl.ds(o, r)], k_v.at[slot, pl.ds(o, r)], sem_kv.at[0, slot]).start(priority=0)
                pltpu.make_async_copy(v_hbm.at[h, pl.ds(o, r)], v_v.at[slot, pl.ds(o, r)], sem_kv.at[1, slot]).start(priority=1 if two_q else 0)

        def wait_k(slot):
            pltpu.make_async_copy(k_v.at[slot], k_v.at[slot], sem_kv.at[0, slot]).wait()

        def wait_v(slot):
            pltpu.make_async_copy(v_v.at[slot], v_v.at[slot], sem_kv.at[1, slot]).wait()

        items = [(awq_hbm, awq_v), (wuk_hbm, wuk_v), (ckv_hbm, ckv_v), (wuv_hbm, wuv_v),
                 (awo_hbm, awo_v), (bwq_hbm, bwq_v), (bwo_hbm, bwo_v)]
        x_cp = pltpu.make_async_copy(x_hbm, x_v, sem_w.at[7])
        g_cp = pltpu.make_async_copy(gate_hbm, gate_v, sem_w.at[8])
        x_cp.start()
        g_cp.start()
        for i, (s_, d_) in enumerate(items):
            add_item(s_, d_, sem_w.at[i])
        for h in range(D):
            add_kv_static(h, h)
        issue_until(LA)

        if not compute:
            x_cp.wait(); g_cp.wait()
            for i, (s_, d_) in enumerate(items):
                need(i)
            issue_until(len(stream))
            def head0(h, c):
                slot = lax.rem(h, NBUF)
                @pl.when(h + D < H)
                def _():
                    start_kv(h + D, lax.rem(h + D, NBUF))
                wait_k(slot); wait_v(slot)
                return c
            lax.fori_loop(0, H, head0, 0)
            out_ref[...] = jnp.zeros_like(out_ref)
            return
        lane = lax.broadcasted_iota(jnp.int32, (128, 4096), 1)
        row = lax.broadcasted_iota(jnp.int32, (128, 4096), 0)
        E = jnp.where((lane >> 5) == row, 1.0, 0.0).astype(BF16)
        dmask = (lane & 31) == (row & 31)

        x_cp.wait()
        g_cp.wait()
        x = x_v[...]
        xf = x.astype(F32)
        gl = jnp.sum(xf * gate_v[...].reshape(1, M).astype(F32), axis=-1, keepdims=True)
        g = jax.nn.sigmoid(gl)

        xb = jnp.broadcast_to(x, (32, M))
        x5 = jnp.concatenate([xb[:, 128 * b:128 * (b + 1)] for b in range(4)], axis=0)
        rep = jnp.dot(x5, E, preferred_element_type=F32)
        lhs = jnp.where(dmask, rep, 0.0).astype(BF16)
        rep4 = jnp.dot(xb[:, 512:640], E[:, :], preferred_element_type=F32)
        lhs4 = jnp.where(dmask[:32], rep4, 0.0).astype(BF16)
        need(0)
        qa = jnp.dot(lhs4, awq_v[pl.ds(4 * 4096, 4096), :], preferred_element_type=F32)
        for b in range(4):
            qa = qa + jnp.dot(lhs[32 * b:32 * (b + 1)], awq_v[pl.ds(b * 4096, 4096), :], preferred_element_type=F32)
        qa = qa.astype(BF16)

        need(1)
        tm = []
        for b in range(4):
            t = lax.dot_general(qa, wuk_v[pl.ds(b * 4096, 4096), :], NT, preferred_element_type=F32)
            tm.append(jnp.where(dmask[:32], t, 0.0).astype(BF16))
        tm4 = jnp.concatenate(tm, axis=0)
        qabs4 = lax.dot_general(tm4, E, NT, preferred_element_type=F32)
        qabs = jnp.concatenate([qabs4[32 * b:32 * (b + 1)] for b in range(4)], axis=1).astype(BF16)

        need(2)
        ckv = ckv_v[...]
        sa = lax.dot_general(qabs, ckv, NT, preferred_element_type=F32) * (DH ** -0.5)
        ma = jnp.max(sa, axis=-1, keepdims=True)
        pa = jnp.exp(sa - ma)
        la = jnp.sum(pa, axis=-1, keepdims=True)
        ca = jnp.dot(pa.astype(BF16), ckv, preferred_element_type=F32) / la
        ca = ca.astype(BF16)

        ca4 = jnp.concatenate([ca[:, 128 * b:128 * (b + 1)] for b in range(4)], axis=0)
        rep = jnp.dot(ca4, E, preferred_element_type=F32)
        lhs = jnp.where(dmask, rep, 0.0).astype(BF16)
        need(3)
        ctx = jnp.dot(lhs[0:32], wuv_v[pl.ds(0, 4096), :], preferred_element_type=F32)
        for b in range(1, 4):
            ctx = ctx + jnp.dot(lhs[32 * b:32 * (b + 1)], wuv_v[pl.ds(b * 4096, 4096), :], preferred_element_type=F32)

        ctx_flat = jnp.concatenate([jnp.broadcast_to(ctx[h:h + 1, :], (8, 128)) for h in range(H)], axis=1).astype(BF16)
        need(4)
        out_a = jnp.dot(ctx_flat, awo_v[...], preferred_element_type=F32)

        need(5)
        x8 = jnp.broadcast_to(x, (8, M))
        qb = jnp.dot(x8, bwq_v[...], preferred_element_type=F32)
        for h in range(H):
            qb_s[h] = qb[:, 128 * h:128 * (h + 1)]
        need(6)

        issue_until(len(stream))
        def head(h, acc):
            slot = lax.rem(h, NBUF)

            @pl.when(h + D < H)
            def _():
                start_kv(h + D, lax.rem(h + D, NBUF))

            q = qb_s[h].astype(BF16)
            wait_k(slot)
            s = lax.dot_general(q, k_v[slot], NT, preferred_element_type=F32) * (DH ** -0.5)
            m = jnp.max(s, axis=-1, keepdims=True)
            p = jnp.exp(s - m)
            l = jnp.sum(p, axis=-1, keepdims=True)
            wait_v(slot)
            o = jnp.dot(p.astype(BF16), v_v[slot], preferred_element_type=F32) / l
            wo = bwo_v[pl.ds(pl.multiple_of(h * DH, DH), DH), :]
            return acc + jnp.dot(o.astype(BF16), wo, preferred_element_type=F32)

        out_b = lax.fori_loop(0, H, head, jnp.zeros((8, M), F32))

        res = g * out_a[0:1] + (1.0 - g) * out_b[0:1]
        out_ref[...] = res.astype(BF16)

    call = pl.pallas_call(
        kernel,
        out_shape=jax.ShapeDtypeStruct((1, M), BF16),
        in_specs=[pl.BlockSpec(memory_space=pl.ANY)] * 11,
        out_specs=pl.BlockSpec(memory_space=pltpu.VMEM),
        scratch_shapes=[
            pltpu.VMEM((1, M), BF16),
            pltpu.VMEM((M,), BF16),
            pltpu.VMEM((S, DC), BF16),
            pltpu.VMEM((M * H, DH), BF16),
            pltpu.VMEM((DC * H, DH), BF16),
            pltpu.VMEM((DC * H, DH), BF16),
            pltpu.VMEM((H * DH, M), BF16),
            pltpu.VMEM((M, H * DH), BF16),
            pltpu.VMEM((H * DH, M), BF16),
            pltpu.VMEM((NBUF, S, DH), BF16),
            pltpu.VMEM((NBUF, S, DH), BF16),
            pltpu.VMEM((H, 8, DH), F32),
            pltpu.SemaphoreType.DMA((9,)),
            pltpu.SemaphoreType.DMA((2, NBUF)),
        ],
        compiler_params=pltpu.CompilerParams(vmem_limit_bytes=110 * 1024 * 1024),
    )

    @jax.jit
    def fn(A_x, A_c_kv, A_w_q, A_w_uk, A_w_uv, A_w_o, B_x, B_k_cache, B_v_cache, B_wq, B_wo, gate_w):
        out = call(
            A_x.reshape(1, M),
            A_c_kv.reshape(S, DC),
            A_w_q.reshape(M * H, DH),
            A_w_uk.reshape(DC * H, DH),
            A_w_uv.reshape(DC * H, DH),
            A_w_o.reshape(H * DH, M),
            B_k_cache.reshape(H, S, DH),
            B_v_cache.reshape(H, S, DH),
            B_wq, B_wo, gate_w)
        return out.reshape(1, 1, M)
    return fn


_fn = _make()


def pallas_gated_mix__compressed_kv_cla__gqa_block_cached__decode_kernel(
    A_x, A_c_kv, A_w_q, A_w_uk, A_w_uv, A_w_o, B_x, B_k_cache, B_v_cache, B_wq, B_wo, gate_w
):
    return _fn(A_x, A_c_kv, A_w_q, A_w_uk, A_w_uv, A_w_o, B_x, B_k_cache, B_v_cache, B_wq, B_wo, gate_w)
```

```python
import numpy as np
import jax
import jax.numpy as jnp
from jax import lax
from jax.experimental import pallas as pl
from jax.experimental.pallas import tpu as pltpu

H, DH, M, DC, S = 32, 128, 640, 512, 4096
F32, BF16 = jnp.float32, jnp.bfloat16
NT = (((1,), (1,)), ((), ()))
CH = 128
NCH = S // CH


def _linear_chunks(rows, cols, w640):
    out = []
    if cols == 4096:
        for b in range(rows // 8):
            out += [(8 * b, 8, 0, 2048), (8 * b, 8, 2048, 2048)]
    elif cols == 640:
        o, k = 0, 0
        while o < rows:
            r = w640[k % len(w640)]
            out.append((o, r, 0, cols))
            o += r
            k += 1
        assert o == rows
    else:
        step = 32 * 1024 // (2 * cols)
        out = [(o, step, 0, cols) for o in range(0, rows, step)]
    return out


def _kv_round(r, STAG):
    return [(i, r // STAG - i, r - STAG * (r // STAG - i)) for i in range(NCH // STAG)]


def _edf_tail(r_end, STAG):
    out = []
    for n in range(2 * H):
        first = max(0, r_end - STAG * n)
        if first < NCH:
            c = list(range(first, NCH))
            a, b = c[:len(c) // 2], c[len(c) // 2:]
            for i in range(max(len(a), len(b))):
                if i < len(a):
                    out.append((n, a[i]))
                if i < len(b):
                    out.append((n, b[i]))
    return out


def _make(LA=72, tick=16, C=40, w640=(24, 24, 24, 24, 32), ns=8, ns5=8, epi=(32, 32, 24, 24, 0), fill=True,
                compA=True, compB=True, vsplit=False, order=(0, 5, 1, 2, 3, 4, 6), barrier='sem0', skip=(), NW=0, wo_rows=32, STAG=4, NSLOT=8, lastthr=False):
    RPH = 2 * STAG
    NLOOP = (2 * H * STAG - C - RPH) // RPH + 1
    R_END = RPH * (NLOOP - 1) + C + RPH
    tail = _edf_tail(R_END, STAG)
    if epi is None:
        rem, epi = len(tail) + NW * (DH // wo_rows), []
        for _h in range(NLOOP, H):
            left = H - 1 - _h
            take = rem if left <= 0 else min(rem, max(24, -(-rem // max(left - 0, 1)) if left <= 2 else 32))
            epi.append(take); rem -= take
        epi = tuple(epi)
    WO0 = H - NW
    wo_tail = [(hh, r0) for hh in range(WO0, H) for r0 in range(0, DH, wo_rows)]
    tail = tail + [(-1, t) for t in wo_tail]
    assert len(epi) == H - NLOOP and sum(epi) == len(tail), (NLOOP, len(tail))
    assert WO0 >= NLOOP
    LAST = 2 * H - 1
    last_first = max(0, R_END - STAG * LAST)
    last_tail = [c for (n, c) in tail if n == LAST]
    NG = 4
    last_groups = [last_tail[i * 8:(i + 1) * 8] for i in range(NG)]
    assert sum(len(g) for g in last_groups) == len(last_tail)

    def kernel(x_hbm, ckv_hbm, awq_hbm, wuk_hbm, wuv_hbm, awo_hbm, k_hbm, v_hbm,
               bwq_hbm, bwo_hbm, gate_hbm,
               out_ref,
               x_v, gate_v, ckv_v, awq_v, wuk_v, wuv_v, awo_v, bwq_v, bwo_v, k_v, v_v,
               qb_s, sem_w, sem_kv, sem_last, sem_bar, sem_wo):
        items = [(awq_hbm, awq_v, 128, ns5), (wuk_hbm, wuk_v, 128, ns), (ckv_hbm, ckv_v, 32, ns), (wuv_hbm, wuv_v, 128, ns),
                 (awo_hbm, awo_v, w640, ns5), (bwq_hbm, bwq_v, 8, ns5), (bwo_hbm, bwo_v, w640, ns5)]
        item_rows = [it[1].shape[0] for it in items]
        item_rows[6] = WO0 * DH

        def w_copy(i, ch):
            src, dst = items[i][0], items[i][1]
            r0, nr, c0, nc = ch
            return pltpu.make_async_copy(src.at[pl.ds(r0, nr), pl.ds(c0, nc)],
                                         dst.at[pl.ds(r0, nr), pl.ds(c0, nc)], sem_w.at[i])

        def kv_copy(head, slot, a, idx, sem=None):
            src, dst = (k_hbm, k_v) if a == 0 else (v_hbm, v_v)
            o = idx * CH
            return pltpu.make_async_copy(src.at[head, pl.ds(o, CH)], dst.at[slot, pl.ds(o, CH)],
                                         sem_kv.at[a, slot] if sem is None else sem)

        stream, item_end, issued = [], {}, [0]
        wch = [_linear_chunks(item_rows[i], it[1].shape[1], w640) for i, it in enumerate(items)]
        witems = []
        for i in order:
            assert len(wch[i]) % NCH == 0, (i, len(wch[i]))
            for j in range(len(wch[i]) // NCH):
                witems.append((i, wch[i][j * NCH:(j + 1) * NCH]))
        NWI = len(witems)
        for r in range(STAG * NWI + C):
            for (slot_i, gi, c) in _kv_round(r, STAG):
                if gi < 0:
                    continue
                q = gi % 2
                if gi < NWI:
                    i, chs = witems[gi]
                    stream.append(lambda _q, i=i, ch=chs[c], q=q: w_copy(i, ch).start(priority=q))
                    item_end[i] = len(stream)
                else:
                    n = gi - NWI
                    stream.append(lambda _q, n=n, c=c, q=q: kv_copy(n // 2, (n // 2) % NSLOT, n % 2, c).start(priority=q))

        def issue_until(n):
            n = min(n, len(stream))
            while issued[0] < n:
                stream[issued[0]](issued[0] % 2)
                issued[0] += 1

        def need(i):
            issue_until(item_end[i] + LA)
            d = items[i][1].at[pl.ds(0, item_rows[i])]
            pltpu.make_async_copy(d, d, sem_w.at[i]).wait()

        tick_id = [0]

        def do_tick():
            tick_id[0] += 1
            if barrier == 'scope':
                with jax.named_scope(f"tick{tick_id[0]}"):
                    issue_until(issued[0] + tick)
            elif barrier == 'sem':
                pl.semaphore_signal(sem_bar.at[0], 1)
                pl.semaphore_wait(sem_bar.at[0], 1)
                issue_until(issued[0] + tick)
            elif barrier == 'sem0':
                pl.semaphore_wait(sem_bar.at[0], 0)
                issue_until(issued[0] + tick)
            else:
                issue_until(issued[0] + tick)

        x_cp = pltpu.make_async_copy(x_hbm, x_v, sem_w.at[7])
        g_cp = pltpu.make_async_copy(gate_hbm, gate_v, sem_w.at[8])
        x_cp.start()
        g_cp.start()
        issue_until(LA)

        def issue_loop(h):
            for j in range(RPH):
                for (i, n, c) in _kv_round(C + j, STAG):
                    head = h + n // 2
                    kv_copy(head, jnp.bitwise_and(head, NSLOT - 1), n % 2, c).start(priority=n % 2)

        tail_pos = [0]

        def last_copy(c):
            g = next(gi for gi, grp in enumerate(last_groups) if c in grp)
            return kv_copy(H - 1, (H - 1) % NSLOT, 1, c, sem=sem_last.at[g])

        def wo_copy(hh, r0):
            return pltpu.make_async_copy(bwo_hbm.at[pl.ds(hh * DH + r0, wo_rows)], bwo_v.at[pl.ds(hh * DH + r0, wo_rows)],
                                         sem_wo.at[hh - WO0])

        def issue_tail(cnt):
            for (n, c) in tail[tail_pos[0]:tail_pos[0] + cnt]:
                q = tail_pos[0] % 2
                if n < 0:
                    wo_copy(*c).start(priority=q)
                elif n == LAST and vsplit:
                    last_copy(c).start(priority=q)
                else:
                    kv_copy(n // 2, (n // 2) % NSLOT, n % 2, c).start(priority=q)
                tail_pos[0] += 1

        def wait_kv(a, slot):
            d = (k_v if a == 0 else v_v).at[slot]
            pltpu.make_async_copy(d, d, sem_kv.at[a, slot]).wait()

        def head(h, acc, static):
            slot = (h % NSLOT) if static else jnp.bitwise_and(h, NSLOT - 1)
            last = static and h == H - 1 and vsplit
            if static:
                issue_tail(epi[h - NLOOP])
            else:
                issue_loop(h)
            if not compB:
                wait_kv(0, slot)
                if last:
                    for c in range(last_first):
                        kv_copy(h, slot, 1, c).wait()
                    for c in last_tail:
                        last_copy(c).wait()
                else:
                    wait_kv(1, slot)
                return acc
            q = qb_s[h].astype(BF16)
            wait_kv(0, slot)
            s = lax.dot_general(q, k_v[slot], NT, preferred_element_type=F32)
            m = jnp.max(s, axis=-1, keepdims=True)
            p = jnp.exp(s - m)
            l = jnp.sum(p, axis=-1, keepdims=True)
            pb = p.astype(BF16)
            if last:
                for c in range(last_first):
                    kv_copy(h, slot, 1, c).wait()
                o = jnp.dot(pb[:, :last_first * CH], v_v[slot, pl.ds(0, last_first * CH), :], preferred_element_type=F32)
                for grp in last_groups:
                    for c in grp:
                        last_copy(c).wait()
                    for c in grp:
                        o = o + jnp.dot(pb[:, c * CH:(c + 1) * CH], v_v[slot, pl.ds(c * CH, CH), :], preferred_element_type=F32)
            else:
                wait_kv(1, slot)
                o = jnp.dot(pb, v_v[slot], preferred_element_type=F32)
            o = (o / l).astype(BF16)
            if static and h >= WO0:
                deferred.append((h, o))
                return acc
            wo = bwo_v[pl.ds(h * DH if static else pl.multiple_of(h * DH, DH), DH), :]
            return acc + jnp.dot(o, wo, preferred_element_type=F32)

        deferred = []

        def run_b():
            out_b = lax.fori_loop(0, NLOOP, lambda h, a: head(h, a, False), jnp.zeros((8, M), F32))
            for h in range(NLOOP, H):
                out_b = head(h, out_b, True)
            if not compB:
                for hh in range(WO0, H):
                    d = bwo_v.at[pl.ds(hh * DH, DH)]
                    pltpu.make_async_copy(d, d, sem_wo.at[hh - WO0]).wait()
            for (hh, o) in deferred:
                d = bwo_v.at[pl.ds(hh * DH, DH)]
                pltpu.make_async_copy(d, d, sem_wo.at[hh - WO0]).wait()
                out_b = out_b + jnp.dot(o, bwo_v[pl.ds(hh * DH, DH), :], preferred_element_type=F32)
            return out_b

        if not compA:
            x_cp.wait(); g_cp.wait()
            for i in order:
                need(i)
            issue_until(len(stream))
            out_ref[...] = run_b()[0:1].astype(BF16)
            return

        lane = lax.broadcasted_iota(jnp.int32, (128, 4096), 1)
        row = lax.broadcasted_iota(jnp.int32, (128, 4096), 0)
        E = jnp.where((lane >> 5) == row, 1.0, 0.0).astype(BF16)
        dmask = (lane & 31) == (row & 31)

        x_cp.wait()
        g_cp.wait()
        x = x_v[...]
        xf = x.astype(F32)
        gl = jnp.sum(xf * gate_v[...].reshape(1, M).astype(F32), axis=-1, keepdims=True)
        g = jax.nn.sigmoid(gl)

        xb = jnp.broadcast_to(x, (32, M))
        x5 = jnp.concatenate([xb[:, 128 * b:128 * (b + 1)] for b in range(5)], axis=0)
        if 0 in skip:
            lhs1 = [jnp.zeros((32, 4096), BF16) for b in range(5)]
        else:
            rep = jnp.dot(x5, E, preferred_element_type=F32)
            lhs1 = [jnp.where(dmask[:32], rep[32 * b:32 * (b + 1)], 0.0).astype(BF16) for b in range(5)]
        need(0)
        qa = jnp.zeros((32, 128), F32) if 1 in skip else None
        for b in range(0 if 1 in skip else 5):
            d = jnp.dot(lhs1[b], awq_v[pl.ds(b * 4096, 4096), :], preferred_element_type=F32)
            qa = d if qa is None else qa + d
            do_tick()
        qa = qa.astype(BF16)

        need(1)
        tm = [jnp.zeros((32, 4096), BF16)] * 4 if 2 in skip else []
        for b in range(0 if 2 in skip else 4):
            t = lax.dot_general(qa, wuk_v[pl.ds(b * 4096, 4096), :], NT, preferred_element_type=F32)
            tm.append(jnp.where(dmask[:32], t, 0.0).astype(BF16))
            do_tick()
        tm4 = jnp.concatenate(tm, axis=0)
        qabs4 = jnp.zeros((128, 128), F32) if 2 in skip else lax.dot_general(tm4, E, NT, preferred_element_type=F32)
        qabs = jnp.concatenate([qabs4[32 * b:32 * (b + 1)] for b in range(4)], axis=1).astype(BF16)

        need(2)
        sa_l = [jnp.zeros((32, 1024), F32)] * 4 if 3 in skip else []
        for kb in range(0 if 3 in skip else 4):
            sa_l.append(lax.dot_general(qabs, ckv_v[pl.ds(kb * 1024, 1024), :], NT, preferred_element_type=F32))
            do_tick()
        sa = jnp.concatenate(sa_l, axis=1) * (DH ** -0.5)
        ma = jnp.max(sa, axis=-1, keepdims=True)
        pa = jnp.exp(sa - ma)
        la = jnp.sum(pa, axis=-1, keepdims=True)
        pab = pa.astype(BF16)
        do_tick()
        ca = jnp.zeros((32, 512), F32) if 3 in skip else None
        for kb in range(0 if 3 in skip else 4):
            d = jnp.dot(pab[:, kb * 1024:(kb + 1) * 1024], ckv_v[pl.ds(kb * 1024, 1024), :], preferred_element_type=F32)
            ca = d if ca is None else ca + d
            do_tick()
        ca = (ca / la).astype(BF16)

        ca4 = jnp.concatenate([ca[:, 128 * b:128 * (b + 1)] for b in range(4)], axis=0)
        if 4 in skip:
            lhs = jnp.zeros((128, 4096), BF16)
        else:
            rep = jnp.dot(ca4, E, preferred_element_type=F32)
            lhs = jnp.where(dmask, rep, 0.0).astype(BF16)
        need(3)
        ctx = jnp.zeros((32, 128), F32) if 4 in skip else None
        for b in range(0 if 4 in skip else 4):
            d = jnp.dot(lhs[32 * b:32 * (b + 1)], wuv_v[pl.ds(b * 4096, 4096), :], preferred_element_type=F32)
            ctx = d if ctx is None else ctx + d
            do_tick()

        ctx_flat = jnp.concatenate([jnp.broadcast_to(ctx[h:h + 1, :], (8, 128)) for h in range(H)], axis=1).astype(BF16)
        need(4)
        out_a = jnp.zeros((8, M), F32) if 5 in skip else None
        for kb in range(0 if 5 in skip else 4):
            d = jnp.dot(ctx_flat[:, kb * 1024:(kb + 1) * 1024], awo_v[pl.ds(kb * 1024, 1024), :], preferred_element_type=F32)
            out_a = d if out_a is None else out_a + d
            do_tick()

        need(5)
        x8 = jnp.broadcast_to(x, (8, M))
        for kb in range(0 if 6 in skip else 4):
            qb = jnp.dot(x8, bwq_v[:, pl.ds(kb * 1024, 1024)], preferred_element_type=F32) * (DH ** -0.5)
            for hh in range(8):
                qb_s[kb * 8 + hh] = qb[:, 128 * hh:128 * (hh + 1)]
            do_tick()
        need(6)
        issue_until(len(stream))

        out_b = run_b()

        res = g * out_a[0:1] + (1.0 - g) * out_b[0:1]
        out_ref[...] = res.astype(BF16)

    call = pl.pallas_call(
        kernel,
        out_shape=jax.ShapeDtypeStruct((1, M), BF16),
        in_specs=[pl.BlockSpec(memory_space=pl.ANY)] * 11,
        out_specs=pl.BlockSpec(memory_space=pltpu.VMEM),
        scratch_shapes=[
            pltpu.VMEM((1, M), BF16),
            pltpu.VMEM((M,), BF16),
            pltpu.VMEM((S, DC), BF16),
            pltpu.VMEM((M * H, DH), BF16),
            pltpu.VMEM((DC * H, DH), BF16),
            pltpu.VMEM((DC * H, DH), BF16),
            pltpu.VMEM((H * DH, M), BF16),
            pltpu.VMEM((M, H * DH), BF16),
            pltpu.VMEM((H * DH, M), BF16),
            pltpu.VMEM((NSLOT, S, DH), BF16),
            pltpu.VMEM((NSLOT, S, DH), BF16),
            pltpu.VMEM((H, 8, DH), F32),
            pltpu.SemaphoreType.DMA((9,)),
            pltpu.SemaphoreType.DMA((2, NSLOT)),
            pltpu.SemaphoreType.DMA((NG,)),
            pltpu.SemaphoreType.REGULAR((1,)),
            pltpu.SemaphoreType.DMA((max(NW, 1),)),
        ],
        compiler_params=pltpu.CompilerParams(vmem_limit_bytes=110 * 1024 * 1024),
    )

    @jax.jit
    def fn(A_x, A_c_kv, A_w_q, A_w_uk, A_w_uv, A_w_o, B_x, B_k_cache, B_v_cache, B_wq, B_wo, gate_w):
        out = call(
            A_x.reshape(1, M),
            A_c_kv.reshape(S, DC),
            A_w_q.reshape(M * H, DH),
            A_w_uk.reshape(DC * H, DH),
            A_w_uv.reshape(DC * H, DH),
            A_w_o.reshape(H * DH, M),
            B_k_cache.reshape(H, S, DH),
            B_v_cache.reshape(H, S, DH),
            B_wq, B_wo, gate_w)
        return out.reshape(1, 1, M)
    return fn


_fn = _make()


def pallas_gated_mix__compressed_kv_cla__gqa_block_cached__decode_kernel(
    A_x, A_c_kv, A_w_q, A_w_uk, A_w_uv, A_w_o, B_x, B_k_cache, B_v_cache, B_wq, B_wo, gate_w
):
    return _fn(A_x, A_c_kv, A_w_q, A_w_uk, A_w_uv, A_w_o, B_x, B_k_cache, B_v_cache, B_wq, B_wo, gate_w)
```

```python
import numpy as np
import jax
import jax.numpy as jnp
from jax import lax
from jax.experimental import pallas as pl
from jax.experimental.pallas import tpu as pltpu

H, DH, M, DC, S = 32, 128, 640, 512, 4096
F32, BF16 = jnp.float32, jnp.bfloat16
NT = (((1,), (1,)), ((), ()))
CH = 128
NCH = S // CH


def _linear_chunks(rows, cols, w640, bwqoff=False):
    out = []
    if cols == 4096:
        for b in range(rows // 8):
            if bwqoff:
                out += [[(8 * b, 8, 0, 1024), (8 * b, 8, 3072, 1024)], (8 * b, 8, 1024, 2048)]
            else:
                out += [(8 * b, 8, 0, 2048), (8 * b, 8, 2048, 2048)]
    elif cols == 640:
        o, k = 0, 0
        while o < rows:
            r = w640[k % len(w640)]
            out.append((o, r, 0, cols))
            o += r
            k += 1
        assert o == rows
    else:
        step = 32 * 1024 // (2 * cols)
        out = [(o, step, 0, cols) for o in range(0, rows, step)]
    return out


def _kv_round(r, STAG):
    return [(i, r // STAG - i, r - STAG * (r // STAG - i)) for i in range(NCH // STAG)]


def _edf_tail(r_end, STAG):
    out = []
    for n in range(2 * H):
        first = max(0, r_end - STAG * n)
        if first < NCH:
            c = list(range(first, NCH))
            a, b = c[:len(c) // 2], c[len(c) // 2:]
            for i in range(max(len(a), len(b))):
                if i < len(a):
                    out.append((n, a[i]))
                if i < len(b):
                    out.append((n, b[i]))
    return out


def _make(LA=72, tick=16, C=40, w640=(24, 24, 24, 24, 32), ns=8, ns5=8, epi=(32, 32, 24, 24, 0), fill=True,
                compA=True, compB=True, vsplit=False, order=(0, 5, 1, 2, 3, 4, 6), barrier='sem0', skip=(), NW=0, wo_rows=32, STAG=4, NSLOT=8, lastthr=False, kvoff=64, bwqoff=True, skip_last=0, semchk=True, bc=True):
    RPH = 2 * STAG
    NLOOP = (2 * H * STAG - C - RPH) // RPH + 1
    R_END = RPH * (NLOOP - 1) + C + RPH
    tail = _edf_tail(R_END, STAG)
    if epi is None:
        rem, epi = len(tail) + NW * (DH // wo_rows), []
        for _h in range(NLOOP, H):
            left = H - 1 - _h
            take = rem if left <= 0 else min(rem, max(24, -(-rem // max(left - 0, 1)) if left <= 2 else 32))
            epi.append(take); rem -= take
        epi = tuple(epi)
    WO0 = H - NW
    wo_tail = [(hh, r0) for hh in range(WO0, H) for r0 in range(0, DH, wo_rows)]
    tail = tail + [(-1, t) for t in wo_tail]
    assert len(epi) == H - NLOOP and sum(epi) == len(tail), (NLOOP, len(tail))
    assert WO0 >= NLOOP
    LAST = 2 * H - 1
    last_first = max(0, R_END - STAG * LAST)
    last_tail = [c for (n, c) in tail if n == LAST]
    NG = 4
    last_groups = [last_tail[i * 8:(i + 1) * 8] for i in range(NG)]
    assert sum(len(g) for g in last_groups) == len(last_tail)

    def kernel(x_hbm, ckv_hbm, awq_hbm, wuk_hbm, wuv_hbm, awo_hbm, k_hbm, v_hbm,
               bwq_hbm, bwo_hbm, gate_hbm,
               out_ref,
               x_v, gate_v, ckv_v, awq_v, wuk_v, wuv_v, awo_v, bwq_v, bwo_v, k_v, v_v,
               qb_s, sem_w, sem_kv, sem_last, sem_bar, sem_wo):
        items = [(awq_hbm, awq_v, 128, ns5), (wuk_hbm, wuk_v, 128, ns), (ckv_hbm, ckv_v, 32, ns), (wuv_hbm, wuv_v, 128, ns),
                 (awo_hbm, awo_v, w640, ns5), (bwq_hbm, bwq_v, 8, ns5), (bwo_hbm, bwo_v, w640, ns5)]
        item_rows = [it[1].shape[0] for it in items]
        item_rows[6] = WO0 * DH

        class _Multi:
            def __init__(self, cps):
                self.cps = cps

            def start(self, priority=0):
                for j, cp in enumerate(self.cps):
                    cp.start(priority=(priority + j) % 2)

            def wait(self):
                for cp in self.cps:
                    cp.wait()

        def w_copy(i, ch):
            src, dst = items[i][0], items[i][1]
            parts = ch if isinstance(ch, list) else [ch]
            return _Multi([pltpu.make_async_copy(src.at[pl.ds(r0, nr), pl.ds(c0, nc)],
                                                 dst.at[pl.ds(r0, nr), pl.ds(c0, nc)], sem_w.at[i])
                           for (r0, nr, c0, nc) in parts])

        def kv_copy(head, slot, a, idx, sem=None):
            src, dst = (k_hbm, k_v) if a == 0 else (v_hbm, v_v)
            sem = sem_kv.at[a, slot] if sem is None else sem
            if kvoff == 0:
                spans = [(idx * CH, CH)]
            elif idx == 0:
                spans = [(0, kvoff), (S - (CH - kvoff), CH - kvoff)]
            else:
                spans = [(kvoff + (idx - 1) * CH, CH)]
            return _Multi([pltpu.make_async_copy(src.at[head, pl.ds(o, n)], dst.at[slot, pl.ds(o, n)], sem)
                           for (o, n) in spans])

        stream, item_end, issued = [], {}, [0]
        wch = [_linear_chunks(item_rows[i], it[1].shape[1], w640, bwqoff) for i, it in enumerate(items)]
        witems = []
        for i in order:
            assert len(wch[i]) % NCH == 0, (i, len(wch[i]))
            for j in range(len(wch[i]) // NCH):
                witems.append((i, wch[i][j * NCH:(j + 1) * NCH]))
        NWI = len(witems)
        for r in range(STAG * NWI + C):
            for (slot_i, gi, c) in _kv_round(r, STAG):
                if gi < 0:
                    continue
                q = gi % 2
                if gi < NWI:
                    i, chs = witems[gi]
                    stream.append(lambda _q, i=i, ch=chs[c], q=q: w_copy(i, ch).start(priority=q))
                    item_end[i] = len(stream)
                else:
                    n = gi - NWI
                    stream.append(lambda _q, n=n, c=c, q=q: kv_copy(n // 2, (n // 2) % NSLOT, n % 2, c).start(priority=q))

        def issue_until(n):
            n = min(n, len(stream))
            while issued[0] < n:
                stream[issued[0]](issued[0] % 2)
                issued[0] += 1

        def need(i):
            issue_until(item_end[i] + LA)
            d = items[i][1].at[pl.ds(0, item_rows[i])]
            pltpu.make_async_copy(d, d, sem_w.at[i]).wait()

        tick_id = [0]

        def do_tick():
            tick_id[0] += 1
            if barrier == 'scope':
                with jax.named_scope(f"tick{tick_id[0]}"):
                    issue_until(issued[0] + tick)
            elif barrier == 'sem':
                pl.semaphore_signal(sem_bar.at[0], 1)
                pl.semaphore_wait(sem_bar.at[0], 1)
                issue_until(issued[0] + tick)
            elif barrier == 'sem0':
                pl.semaphore_wait(sem_bar.at[0], 0)
                issue_until(issued[0] + tick)
            else:
                issue_until(issued[0] + tick)

        x_cp = pltpu.make_async_copy(x_hbm, x_v, sem_w.at[7])
        g_cp = pltpu.make_async_copy(gate_hbm, gate_v, sem_w.at[8])
        x_cp.start()
        g_cp.start()
        issue_until(LA)

        def issue_loop(h):
            for j in range(RPH):
                for (i, n, c) in _kv_round(C + j, STAG):
                    head = h + n // 2
                    kv_copy(head, jnp.bitwise_and(head, NSLOT - 1), n % 2, c).start(priority=n % 2)

        tail_pos = [0]

        def last_copy(c):
            g = next(gi for gi, grp in enumerate(last_groups) if c in grp)
            return kv_copy(H - 1, (H - 1) % NSLOT, 1, c, sem=sem_last.at[g])

        def wo_copy(hh, r0):
            return pltpu.make_async_copy(bwo_hbm.at[pl.ds(hh * DH + r0, wo_rows)], bwo_v.at[pl.ds(hh * DH + r0, wo_rows)],
                                         sem_wo.at[hh - WO0])

        def issue_tail(cnt):
            for (n, c) in tail[tail_pos[0]:tail_pos[0] + cnt]:
                q = tail_pos[0] % 2
                if n < 0:
                    wo_copy(*c).start(priority=q)
                elif n == LAST and vsplit:
                    last_copy(c).start(priority=q)
                else:
                    kv_copy(n // 2, (n // 2) % NSLOT, n % 2, c).start(priority=q)
                tail_pos[0] += 1

        def wait_kv(a, slot):
            d = (k_v if a == 0 else v_v).at[slot]
            pltpu.make_async_copy(d, d, sem_kv.at[a, slot]).wait()

        def head(h, acc, static):
            slot = (h % NSLOT) if static else jnp.bitwise_and(h, NSLOT - 1)
            last = static and h == H - 1 and vsplit
            if static:
                issue_tail(epi[h - NLOOP])
            else:
                issue_loop(h)
            if (not compB) or (static and h >= H - skip_last):
                wait_kv(0, slot)
                if last:
                    for c in range(last_first):
                        kv_copy(h, slot, 1, c).wait()
                    for c in last_tail:
                        last_copy(c).wait()
                else:
                    wait_kv(1, slot)
                return acc
            q = qb_s[h].astype(BF16)
            wait_kv(0, slot)
            s = lax.dot_general(q, k_v[slot], NT, preferred_element_type=F32)
            m = jnp.max(s, axis=-1, keepdims=True)
            p = jnp.exp(s - m)
            l = jnp.sum(p, axis=-1, keepdims=True)
            pb = p.astype(BF16)
            if last:
                for c in range(last_first):
                    kv_copy(h, slot, 1, c).wait()
                o = jnp.dot(pb[:, :last_first * CH], v_v[slot, pl.ds(0, last_first * CH), :], preferred_element_type=F32)
                for grp in last_groups:
                    for c in grp:
                        last_copy(c).wait()
                    for c in grp:
                        o = o + jnp.dot(pb[:, c * CH:(c + 1) * CH], v_v[slot, pl.ds(c * CH, CH), :], preferred_element_type=F32)
            else:
                wait_kv(1, slot)
                o = jnp.dot(pb, v_v[slot], preferred_element_type=F32)
            o = (o / l).astype(BF16)
            if static and h >= WO0:
                deferred.append((h, o))
                return acc
            wo = bwo_v[pl.ds(h * DH if static else pl.multiple_of(h * DH, DH), DH), :]
            return acc + jnp.dot(o, wo, preferred_element_type=F32)

        deferred = []

        def run_b():
            out_b = lax.fori_loop(0, NLOOP, lambda h, a: head(h, a, False), jnp.zeros((8, M), F32))
            for h in range(NLOOP, H):
                out_b = head(h, out_b, True)
            if not compB:
                for hh in range(WO0, H):
                    d = bwo_v.at[pl.ds(hh * DH, DH)]
                    pltpu.make_async_copy(d, d, sem_wo.at[hh - WO0]).wait()
            for (hh, o) in deferred:
                d = bwo_v.at[pl.ds(hh * DH, DH)]
                pltpu.make_async_copy(d, d, sem_wo.at[hh - WO0]).wait()
                out_b = out_b + jnp.dot(o, bwo_v[pl.ds(hh * DH, DH), :], preferred_element_type=F32)
            return out_b

        if not compA:
            x_cp.wait(); g_cp.wait()
            for i in order:
                need(i)
            issue_until(len(stream))
            out_ref[...] = run_b()[0:1].astype(BF16)
            return

        lane = lax.broadcasted_iota(jnp.int32, (128, 4096), 1)
        row = lax.broadcasted_iota(jnp.int32, (128, 4096), 0)
        E = jnp.where((lane >> 5) == row, 1.0, 0.0).astype(BF16)
        dmask = (lane & 31) == (row & 31)

        x_cp.wait()
        g_cp.wait()
        x = x_v[...]
        xf = x.astype(F32)
        gl = jnp.sum(xf * gate_v[...].reshape(1, M).astype(F32), axis=-1, keepdims=True)
        g = jax.nn.sigmoid(gl)

        xb = jnp.broadcast_to(x, (32, M))
        x5 = jnp.concatenate([xb[:, 128 * b:128 * (b + 1)] for b in range(5)], axis=0)
        if 0 in skip:
            lhs1 = [jnp.zeros((32, 4096), BF16) for b in range(5)]
        else:
            rep = jnp.dot(x5, E, preferred_element_type=F32)
            lhs1 = [jnp.where(dmask[:32], rep[32 * b:32 * (b + 1)], 0.0).astype(BF16) for b in range(5)]
        need(0)
        qa = jnp.zeros((32, 128), F32) if 1 in skip else None
        for b in range(0 if 1 in skip else 5):
            d = jnp.dot(lhs1[b], awq_v[pl.ds(b * 4096, 4096), :], preferred_element_type=F32)
            qa = d if qa is None else qa + d
            do_tick()
        qa = qa.astype(BF16)

        need(1)
        tm = [jnp.zeros((32, 4096), BF16)] * 4 if 2 in skip else []
        for b in range(0 if 2 in skip else 4):
            t = lax.dot_general(qa, wuk_v[pl.ds(b * 4096, 4096), :], NT, preferred_element_type=F32)
            tm.append(jnp.where(dmask[:32], t, 0.0).astype(BF16))
            do_tick()
        tm4 = jnp.concatenate(tm, axis=0)
        qabs4 = jnp.zeros((128, 128), F32) if 2 in skip else lax.dot_general(tm4, E, NT, preferred_element_type=F32)
        qabs = jnp.concatenate([qabs4[32 * b:32 * (b + 1)] for b in range(4)], axis=1).astype(BF16)

        need(2)
        sa_l = [jnp.zeros((32, 1024), F32)] * 4 if 3 in skip else []
        for kb in range(0 if 3 in skip else 4):
            sa_l.append(lax.dot_general(qabs, ckv_v[pl.ds(kb * 1024, 1024), :], NT, preferred_element_type=F32))
            do_tick()
        sa = jnp.concatenate(sa_l, axis=1) * (DH ** -0.5)
        ma = jnp.max(sa, axis=-1, keepdims=True)
        pa = jnp.exp(sa - ma)
        la = jnp.sum(pa, axis=-1, keepdims=True)
        pab = pa.astype(BF16)
        do_tick()
        ca = jnp.zeros((32, 512), F32) if 3 in skip else None
        for kb in range(0 if 3 in skip else 4):
            d = jnp.dot(pab[:, kb * 1024:(kb + 1) * 1024], ckv_v[pl.ds(kb * 1024, 1024), :], preferred_element_type=F32)
            ca = d if ca is None else ca + d
            do_tick()
        ca = (ca / la).astype(BF16)

        ca4 = jnp.concatenate([ca[:, 128 * b:128 * (b + 1)] for b in range(4)], axis=0)
        if 4 in skip:
            lhs = jnp.zeros((128, 4096), BF16)
        else:
            rep = jnp.dot(ca4, E, preferred_element_type=F32)
            lhs = jnp.where(dmask, rep, 0.0).astype(BF16)
        need(3)
        ctx = jnp.zeros((32, 128), F32) if 4 in skip else None
        for b in range(0 if 4 in skip else 4):
            d = jnp.dot(lhs[32 * b:32 * (b + 1)], wuv_v[pl.ds(b * 4096, 4096), :], preferred_element_type=F32)
            ctx = d if ctx is None else ctx + d
            do_tick()

        ctx_flat = jnp.concatenate([jnp.broadcast_to(ctx[h:h + 1, :], (8, 128)) for h in range(H)], axis=1).astype(BF16)
        need(4)
        out_a = jnp.zeros((8, M), F32) if 5 in skip else None
        for kb in range(0 if 5 in skip else 4):
            d = jnp.dot(ctx_flat[:, kb * 1024:(kb + 1) * 1024], awo_v[pl.ds(kb * 1024, 1024), :], preferred_element_type=F32)
            out_a = d if out_a is None else out_a + d
            do_tick()

        need(5)
        x8 = jnp.broadcast_to(x, (8, M))
        for kb in range(0 if 6 in skip else 4):
            qb = jnp.dot(x8, bwq_v[:, pl.ds(kb * 1024, 1024)], preferred_element_type=F32) * (DH ** -0.5)
            for hh in range(8):
                qb_s[kb * 8 + hh] = qb[:, 128 * hh:128 * (hh + 1)]
            do_tick()
        need(6)
        issue_until(len(stream))

        out_b = run_b()

        res = g * out_a[0:1] + (1.0 - g) * out_b[0:1]
        out_ref[...] = res.astype(BF16)

    call = pl.pallas_call(
        kernel,
        out_shape=jax.ShapeDtypeStruct((1, M), BF16),
        in_specs=[pl.BlockSpec(memory_space=pl.ANY)] * 11,
        out_specs=pl.BlockSpec(memory_space=pltpu.VMEM),
        scratch_shapes=[
            pltpu.VMEM((1, M), BF16),
            pltpu.VMEM((M,), BF16),
            pltpu.VMEM((S, DC), BF16),
            pltpu.VMEM((M * H, DH), BF16),
            pltpu.VMEM((DC * H, DH), BF16),
            pltpu.VMEM((DC * H, DH), BF16),
            pltpu.VMEM((H * DH, M), BF16),
            pltpu.VMEM((M, H * DH), BF16),
            pltpu.VMEM((H * DH, M), BF16),
            pltpu.VMEM((NSLOT, S, DH), BF16),
            pltpu.VMEM((NSLOT, S, DH), BF16),
            pltpu.VMEM((H, 8, DH), F32),
            pltpu.SemaphoreType.DMA((9,)),
            pltpu.SemaphoreType.DMA((2, NSLOT)),
            pltpu.SemaphoreType.DMA((NG,)),
            pltpu.SemaphoreType.REGULAR((1,)),
            pltpu.SemaphoreType.DMA((max(NW, 1),)),
        ],
        compiler_params=pltpu.CompilerParams(vmem_limit_bytes=110 * 1024 * 1024, disable_semaphore_checks=not semchk, disable_bounds_checks=not bc),
    )

    @jax.jit
    def fn(A_x, A_c_kv, A_w_q, A_w_uk, A_w_uv, A_w_o, B_x, B_k_cache, B_v_cache, B_wq, B_wo, gate_w):
        out = call(
            A_x.reshape(1, M),
            A_c_kv.reshape(S, DC),
            A_w_q.reshape(M * H, DH),
            A_w_uk.reshape(DC * H, DH),
            A_w_uv.reshape(DC * H, DH),
            A_w_o.reshape(H * DH, M),
            B_k_cache.reshape(H, S, DH),
            B_v_cache.reshape(H, S, DH),
            B_wq, B_wo, gate_w)
        return out.reshape(1, 1, M)
    return fn


_fn = _make()


def pallas_gated_mix__compressed_kv_cla__gqa_block_cached__decode_kernel(
    A_x, A_c_kv, A_w_q, A_w_uk, A_w_uv, A_w_o, B_x, B_k_cache, B_v_cache, B_wq, B_wo, gate_w
):
    return _fn(A_x, A_c_kv, A_w_q, A_w_uk, A_w_uv, A_w_o, B_x, B_k_cache, B_v_cache, B_wq, B_wo, gate_w)
```

```python
import numpy as np
import jax
import jax.numpy as jnp
from jax import lax
from jax.experimental import pallas as pl
from jax.experimental.pallas import tpu as pltpu

H, DH, M, DC, S = 32, 128, 640, 512, 4096
F32, BF16 = jnp.float32, jnp.bfloat16
NT = (((1,), (1,)), ((), ()))
SCALE = DH ** -0.5

CH = 128
NCH = S // CH
STAG = 4
NACT = NCH // STAG
RPH = 2 * STAG
NSLOT = 8


def _linear_chunks(rows, cols, shift16k, w640):
    out = []
    if cols == H * DH:
        for b in range(rows // 8):
            if shift16k:
                out += [[(8 * b, 8, 0, 1024), (8 * b, 8, 3072, 1024)], [(8 * b, 8, 1024, 2048)]]
            else:
                out += [[(8 * b, 8, 0, 2048)], [(8 * b, 8, 2048, 2048)]]
    elif cols == M:
        o = k = 0
        while o < rows:
            r = w640[k % len(w640)]
            out.append([(o, r, 0, cols)])
            o += r
            k += 1
        assert o == rows
    else:
        step = 32 * 1024 // (2 * cols)
        out = [[(o, step, 0, cols)] for o in range(0, rows, step)]
    return out


def _round(r):
    return [(r // STAG - i, r - STAG * (r // STAG - i)) for i in range(NACT)]


def _tail(r_end, k_first):
    order = list(range(2 * H))
    if k_first:
        order[-3], order[-2] = order[-2], order[-3]
    out = []
    for n in order:
        first = max(0, r_end - STAG * n)
        if first < NCH:
            c = list(range(first, NCH))
            a, b = c[:len(c) // 2], c[len(c) // 2:]
            for i in range(max(len(a), len(b))):
                if i < len(a):
                    out.append((n, a[i]))
                if i < len(b):
                    out.append((n, b[i]))
    return out


def _make(LA=72, tick=16, C=40, w640=(24, 24, 24, 24, 32), epi=(32, 32, 24, 24, 0), kvoff=64,
                bwq_shift=True, qb_early=False, k_first=True, kv_both=False):
    NLOOP = (2 * H * STAG - C - RPH) // RPH + 1
    R_END = RPH * (NLOOP - 1) + C + RPH
    tail = _tail(R_END, k_first)
    assert len(epi) == H - NLOOP and sum(epi) == len(tail), (NLOOP, len(tail))
    AWQ, BWQ, WUK, CKV, WUV, AWO, BWO = range(7)

    def kernel(x_hbm, ckv_hbm, awq_hbm, wuk_hbm, wuv_hbm, awo_hbm, k_hbm, v_hbm, bwq_hbm, bwo_hbm, gate_hbm,
               out_ref,
               x_v, gate_v, ckv_v, awq_v, wuk_v, wuv_v, awo_v, bwq_v, bwo_v, k_v, v_v, qb_s):
        items = [(awq_hbm, awq_v), (bwq_hbm, bwq_v), (wuk_hbm, wuk_v), (ckv_hbm, ckv_v), (wuv_hbm, wuv_v),
                 (awo_hbm, awo_v), (bwo_hbm, bwo_v)]

        def decode(sem_kv, sem_bar):
            def kv_copies(head, slot, a, idx):
                src, dst = (k_hbm, k_v) if a == 0 else (v_hbm, v_v)
                if kvoff == 0:
                    spans = [(idx * CH, CH)]
                elif idx == 0:
                    spans = [(0, kvoff), (S - (CH - kvoff), CH - kvoff)]
                else:
                    spans = [(kvoff + (idx - 1) * CH, CH)]
                sem = sem_kv.at[0 if kv_both else a, slot]
                return [pltpu.make_async_copy(src.at[head, pl.ds(o, n)], dst.at[slot, pl.ds(o, n)], sem)
                        for (o, n) in spans]

            def start_all(cps, q):
                for j, cp in enumerate(cps):
                    cp.start(priority=(q + j) % 2)

            def wait_kv(a, slot):
                if kv_both:
                    if a == 0:
                        for buf in (k_v, v_v):
                            d = buf.at[slot]
                            pltpu.make_async_copy(d, d, sem_kv.at[0, slot]).wait()
                else:
                    d = (k_v if a == 0 else v_v).at[slot]
                    pltpu.make_async_copy(d, d, sem_kv.at[a, slot]).wait()

            def prologue(sem_w):
                def w_copies(i, piece):
                    src, dst = items[i]
                    return [pltpu.make_async_copy(src.at[pl.ds(r0, nr), pl.ds(c0, nc)],
                                                  dst.at[pl.ds(r0, nr), pl.ds(c0, nc)], sem_w.at[i])
                            for (r0, nr, c0, nc) in piece]

                stream, item_end, issued = [], {}, [0]
                witems = []
                for i, (src, dst) in enumerate(items):
                    ch = _linear_chunks(dst.shape[0], dst.shape[1], bwq_shift and i == BWQ, w640)
                    assert len(ch) % NCH == 0
                    witems += [(i, ch[j * NCH:(j + 1) * NCH]) for j in range(len(ch) // NCH)]
                nwi = len(witems)
                for r in range(STAG * nwi + C):
                    for (g, c) in _round(r):
                        if g < 0:
                            continue
                        if g < nwi:
                            i, ch = witems[g]
                            stream.append(lambda i=i, p=ch[c], q=g % 2: start_all(w_copies(i, p), q))
                            item_end[i] = len(stream)
                        else:
                            n = g - nwi
                            stream.append(lambda n=n, c=c, q=g % 2:
                                          start_all(kv_copies(n // 2, (n // 2) % NSLOT, n % 2, c), q))

                def issue_until(n):
                    n = min(n, len(stream))
                    while issued[0] < n:
                        stream[issued[0]]()
                        issued[0] += 1

                def need(i):
                    issue_until(item_end[i] + LA)
                    d = items[i][1]
                    pltpu.make_async_copy(d, d, sem_w.at[i]).wait()

                def do_tick():
                    pl.semaphore_signal(sem_bar.at[0], 1)
                    pl.semaphore_wait(sem_bar.at[0], 1)
                    issue_until(issued[0] + tick)

                x_cp = pltpu.make_async_copy(x_hbm, x_v, sem_w.at[7])
                g_cp = pltpu.make_async_copy(gate_hbm, gate_v, sem_w.at[8])
                x_cp.start()
                g_cp.start()
                issue_until(LA)

                lane = lax.broadcasted_iota(jnp.int32, (128, 4096), 1)
                row = lax.broadcasted_iota(jnp.int32, (128, 4096), 0)
                E = jnp.where((lane >> 5) == row, 1.0, 0.0).astype(BF16)
                dmask = (lane & 31) == (row & 31)

                x_cp.wait()
                g_cp.wait()
                x = x_v[...]
                gl = jnp.sum(x.astype(F32) * gate_v[...].reshape(1, M).astype(F32), axis=-1, keepdims=True)
                g = jax.nn.sigmoid(gl)

                xb = jnp.broadcast_to(x, (32, M))
                x5 = jnp.concatenate([xb[:, 128 * b:128 * (b + 1)] for b in range(5)], axis=0)
                rep = jnp.dot(x5, E, preferred_element_type=F32)
                lhs1 = [jnp.where(dmask[:32], rep[32 * b:32 * (b + 1)], 0.0).astype(BF16) for b in range(5)]
                need(AWQ)
                qa = None
                for b in range(5):
                    d = jnp.dot(lhs1[b], awq_v[pl.ds(b * 4096, 4096), :], preferred_element_type=F32)
                    qa = d if qa is None else qa + d
                    do_tick()
                qa = qa.astype(BF16)

                def q_proj_b():
                    need(BWQ)
                    x8 = jnp.broadcast_to(x, (8, M))
                    for kb in range(4):
                        qb = jnp.dot(x8, bwq_v[:, pl.ds(kb * 1024, 1024)], preferred_element_type=F32) * SCALE
                        for hh in range(8):
                            qb_s[kb * 8 + hh] = qb[:, 128 * hh:128 * (hh + 1)]
                        do_tick()

                if qb_early:
                    q_proj_b()

                need(WUK)
                tm = []
                for b in range(4):
                    t = lax.dot_general(qa, wuk_v[pl.ds(b * 4096, 4096), :], NT, preferred_element_type=F32)
                    tm.append(jnp.where(dmask[:32], t, 0.0).astype(BF16))
                    do_tick()
                qabs4 = lax.dot_general(jnp.concatenate(tm, axis=0), E, NT, preferred_element_type=F32)
                qabs = jnp.concatenate([qabs4[32 * b:32 * (b + 1)] for b in range(4)], axis=1).astype(BF16)

                need(CKV)
                sa_l = []
                for kb in range(4):
                    sa_l.append(lax.dot_general(qabs, ckv_v[pl.ds(kb * 1024, 1024), :], NT,
                                                preferred_element_type=F32))
                    do_tick()
                sa = jnp.concatenate(sa_l, axis=1) * SCALE
                pa = jnp.exp(sa - jnp.max(sa, axis=-1, keepdims=True))
                la = jnp.sum(pa, axis=-1, keepdims=True)
                pab = pa.astype(BF16)
                do_tick()
                ca = None
                for kb in range(4):
                    d = jnp.dot(pab[:, kb * 1024:(kb + 1) * 1024], ckv_v[pl.ds(kb * 1024, 1024), :],
                                preferred_element_type=F32)
                    ca = d if ca is None else ca + d
                    do_tick()
                ca = (ca / la).astype(BF16)

                ca4 = jnp.concatenate([ca[:, 128 * b:128 * (b + 1)] for b in range(4)], axis=0)
                lhs = jnp.where(dmask, jnp.dot(ca4, E, preferred_element_type=F32), 0.0).astype(BF16)
                need(WUV)
                ctx = None
                for b in range(4):
                    d = jnp.dot(lhs[32 * b:32 * (b + 1)], wuv_v[pl.ds(b * 4096, 4096), :], preferred_element_type=F32)
                    ctx = d if ctx is None else ctx + d
                    do_tick()

                ctx_flat = jnp.concatenate([jnp.broadcast_to(ctx[h:h + 1, :], (8, 128)) for h in range(H)],
                                           axis=1).astype(BF16)
                need(AWO)
                out_a = None
                for kb in range(4):
                    d = jnp.dot(ctx_flat[:, kb * 1024:(kb + 1) * 1024], awo_v[pl.ds(kb * 1024, 1024), :],
                                preferred_element_type=F32)
                    out_a = d if out_a is None else out_a + d
                    do_tick()

                if not qb_early:
                    q_proj_b()
                need(BWO)
                issue_until(len(stream))
                return g, out_a

            g, out_a = pl.run_scoped(prologue, pltpu.SemaphoreType.DMA((9,)))

            tail_pos = [0]

            def issue_tail(cnt):
                for (n, c) in tail[tail_pos[0]:tail_pos[0] + cnt]:
                    start_all(kv_copies(n // 2, (n // 2) % NSLOT, n % 2, c), tail_pos[0] % 2)
                    tail_pos[0] += 1

            def issue_loop(h):
                for j in range(RPH):
                    for (n, c) in _round(C + j):
                        head = h + n // 2
                        start_all(kv_copies(head, jnp.bitwise_and(head, NSLOT - 1), n % 2, c), n % 2)

            def scores(h, slot):
                q = qb_s[h].astype(BF16)
                wait_kv(0, slot)
                s = lax.dot_general(q, k_v[slot], NT, preferred_element_type=F32)
                p = jnp.exp(s - jnp.max(s, axis=-1, keepdims=True))
                return p.astype(BF16), jnp.sum(p, axis=-1, keepdims=True)

            def values(h, slot, pb, l, acc, static):
                wait_kv(1, slot)
                o = (jnp.dot(pb, v_v[slot], preferred_element_type=F32) / l).astype(BF16)
                wo = bwo_v[pl.ds(h * DH if static else pl.multiple_of(h * DH, DH), DH), :]
                return acc + jnp.dot(o, wo, preferred_element_type=F32)

            def body(h, acc):
                slot = jnp.bitwise_and(h, NSLOT - 1)
                issue_loop(h)
                pb, l = scores(h, slot)
                return values(h, slot, pb, l, acc, False)

            out_b = lax.fori_loop(0, NLOOP, body, jnp.zeros((8, M), F32))
            last2 = H - 2 if k_first else H
            for h in range(NLOOP, last2):
                issue_tail(epi[h - NLOOP])
                pb, l = scores(h, h % NSLOT)
                out_b = values(h, h % NSLOT, pb, l, out_b, True)
            if k_first:
                issue_tail(epi[H - 2 - NLOOP] + epi[H - 1 - NLOOP])
                p0, l0 = scores(H - 2, (H - 2) % NSLOT)
                p1, l1 = scores(H - 1, (H - 1) % NSLOT)
                out_b = values(H - 2, (H - 2) % NSLOT, p0, l0, out_b, True)
                out_b = values(H - 1, (H - 1) % NSLOT, p1, l1, out_b, True)
            return g * out_a[0:1] + (1.0 - g) * out_b[0:1]

        res = pl.run_scoped(decode, pltpu.SemaphoreType.DMA((1 if kv_both else 2, NSLOT)),
                            pltpu.SemaphoreType.REGULAR((1,)))
        out_ref[...] = res.astype(BF16)

    call = pl.pallas_call(
        kernel,
        out_shape=jax.ShapeDtypeStruct((1, M), BF16),
        in_specs=[pl.BlockSpec(memory_space=pl.ANY)] * 11,
        out_specs=pl.BlockSpec(memory_space=pltpu.VMEM),
        scratch_shapes=[
            pltpu.VMEM((1, M), BF16),
            pltpu.VMEM((M,), BF16),
            pltpu.VMEM((S, DC), BF16),
            pltpu.VMEM((M * H, DH), BF16),
            pltpu.VMEM((DC * H, DH), BF16),
            pltpu.VMEM((DC * H, DH), BF16),
            pltpu.VMEM((H * DH, M), BF16),
            pltpu.VMEM((M, H * DH), BF16),
            pltpu.VMEM((H * DH, M), BF16),
            pltpu.VMEM((NSLOT, S, DH), BF16),
            pltpu.VMEM((NSLOT, S, DH), BF16),
            pltpu.VMEM((H, 8, DH), F32),
        ],
        compiler_params=pltpu.CompilerParams(vmem_limit_bytes=110 * 1024 * 1024),
    )

    @jax.jit
    def fn(A_x, A_c_kv, A_w_q, A_w_uk, A_w_uv, A_w_o, B_x, B_k_cache, B_v_cache, B_wq, B_wo, gate_w):
        out = call(
            A_x.reshape(1, M),
            A_c_kv.reshape(S, DC),
            A_w_q.reshape(M * H, DH),
            A_w_uk.reshape(DC * H, DH),
            A_w_uv.reshape(DC * H, DH),
            A_w_o.reshape(H * DH, M),
            B_k_cache.reshape(H, S, DH),
            B_v_cache.reshape(H, S, DH),
            B_wq, B_wo, gate_w)
        return out.reshape(1, 1, M)
    return fn


_fn = _make()


def pallas_gated_mix__compressed_kv_cla__gqa_block_cached__decode_kernel(
    A_x, A_c_kv, A_w_q, A_w_uk, A_w_uv, A_w_o, B_x, B_k_cache, B_v_cache, B_wq, B_wo, gate_w
):
    return _fn(A_x, A_c_kv, A_w_q, A_w_uk, A_w_uv, A_w_o, B_x, B_k_cache, B_v_cache, B_wq, B_wo, gate_w)
```

```python
import numpy as np
import jax
import jax.numpy as jnp
from jax import lax
from jax.experimental import pallas as pl
from jax.experimental.pallas import tpu as pltpu

H, DH, M, DC, S = 32, 128, 640, 512, 4096
F32, BF16 = jnp.float32, jnp.bfloat16
NT = (((1,), (1,)), ((), ()))
SCALE = DH ** -0.5

CH = 128
NCH = S // CH
STAG = 4
NACT = NCH // STAG
RPH = 2 * STAG
NSLOT = 8
KV_OFF = 64
AHEAD = 40
LOOK = 72
TICK = 16
EPI = (32, 32, 24, 24, 0)
ROWS640 = (24, 24, 24, 24, 32)

NLOOP = (2 * H * STAG - AHEAD - RPH) // RPH + 1
R_END = RPH * (NLOOP - 1) + AHEAD + RPH


def _linear_pieces(rows, cols):
    out = []
    if cols == H * DH:
        for b in range(rows // 8):
            out += [[(8 * b, 8, 0, 1024), (8 * b, 8, 3072, 1024)], [(8 * b, 8, 1024, 2048)]]
    elif cols == M:
        o = k = 0
        while o < rows:
            r = ROWS640[k % len(ROWS640)]
            out.append([(o, r, 0, cols)])
            o += r
            k += 1
        assert o == rows
    else:
        step = 32 * 1024 // (2 * cols)
        out = [[(o, step, 0, cols)] for o in range(0, rows, step)]
    assert len(out) % NCH == 0
    return out


def _round(r):
    return [(r // STAG - i, r - STAG * (r // STAG - i)) for i in range(NACT)]


def _tail_order():
    order = list(range(2 * H))
    order[-3], order[-2] = order[-2], order[-3]
    out = []
    for n in order:
        first = max(0, R_END - STAG * n)
        if first < NCH:
            c = list(range(first, NCH))
            a, b = c[:len(c) // 2], c[len(c) // 2:]
            for i in range(max(len(a), len(b))):
                if i < len(a):
                    out.append((n, a[i]))
                if i < len(b):
                    out.append((n, b[i]))
    return out


def _kernel(x_hbm, ckv_hbm, awq_hbm, wuk_hbm, wuv_hbm, awo_hbm, k_hbm, v_hbm, bwq_hbm, bwo_hbm, gate_hbm,
            out_ref,
            x_v, gate_v, ckv_v, awq_v, wuk_v, wuv_v, awo_v, bwq_v, bwo_v, k_v, v_v, qb_s):
    AWQ, BWQ, WUK, CKV, WUV, AWO, BWO = range(7)
    weights = [(awq_hbm, awq_v), (bwq_hbm, bwq_v), (wuk_hbm, wuk_v), (ckv_hbm, ckv_v), (wuv_hbm, wuv_v),
               (awo_hbm, awo_v), (bwo_hbm, bwo_v)]
    tail = _tail_order()
    assert len(EPI) == H - NLOOP and sum(EPI) == len(tail)

    def start_all(copies, queue):
        for j, cp in enumerate(copies):
            cp.start(priority=(queue + j) % 2)

    def decode(sem_kv, sem_fence):
        def kv_copies(head, slot, a, pos):
            src, dst = (k_hbm, k_v) if a == 0 else (v_hbm, v_v)
            if pos == 0:
                spans = [(0, KV_OFF), (S - (CH - KV_OFF), CH - KV_OFF)]
            else:
                spans = [(KV_OFF + (pos - 1) * CH, CH)]
            return [pltpu.make_async_copy(src.at[head, pl.ds(o, n)], dst.at[slot, pl.ds(o, n)], sem_kv.at[a, slot])
                    for (o, n) in spans]

        def wait_kv(a, slot):
            d = (k_v if a == 0 else v_v).at[slot]
            pltpu.make_async_copy(d, d, sem_kv.at[a, slot]).wait()

        def prologue(sem_w):
            def w_copies(i, piece):
                src, dst = weights[i]
                return [pltpu.make_async_copy(src.at[pl.ds(r0, nr), pl.ds(c0, nc)],
                                              dst.at[pl.ds(r0, nr), pl.ds(c0, nc)], sem_w.at[i])
                        for (r0, nr, c0, nc) in piece]

            w_items = []
            for i, (_, dst) in enumerate(weights):
                pieces = _linear_pieces(*dst.shape)
                w_items += [(i, pieces[j:j + NCH]) for j in range(0, len(pieces), NCH)]
            n_w = len(w_items)
            stream, last_piece, issued = [], {}, [0]
            for r in range(STAG * n_w + AHEAD):
                for (g, pos) in _round(r):
                    if g < 0:
                        continue
                    if g < n_w:
                        i, pieces = w_items[g]
                        stream.append(lambda i=i, p=pieces[pos], q=g % 2: start_all(w_copies(i, p), q))
                        last_piece[i] = len(stream)
                    else:
                        n = g - n_w
                        stream.append(lambda n=n, pos=pos, q=g % 2:
                                      start_all(kv_copies(n // 2, (n // 2) % NSLOT, n % 2, pos), q))

            def issue_until(n):
                n = min(n, len(stream))
                while issued[0] < n:
                    stream[issued[0]]()
                    issued[0] += 1

            def need(i):
                issue_until(last_piece[i] + LOOK)
                d = weights[i][1]
                pltpu.make_async_copy(d, d, sem_w.at[i]).wait()

            def tick():
                pl.semaphore_signal(sem_fence.at[0], 1)
                pl.semaphore_wait(sem_fence.at[0], 1)
                issue_until(issued[0] + TICK)

            x_cp = pltpu.make_async_copy(x_hbm, x_v, sem_w.at[7])
            g_cp = pltpu.make_async_copy(gate_hbm, gate_v, sem_w.at[8])
            x_cp.start()
            g_cp.start()
            issue_until(LOOK)

            lane = lax.broadcasted_iota(jnp.int32, (128, 4096), 1)
            row = lax.broadcasted_iota(jnp.int32, (128, 4096), 0)
            E = jnp.where((lane >> 5) == row, 1.0, 0.0).astype(BF16)
            diag = (lane & 31) == (row & 31)

            x_cp.wait()
            g_cp.wait()
            x = x_v[...]
            logit = jnp.sum(x.astype(F32) * gate_v[...].reshape(1, M).astype(F32), axis=-1, keepdims=True)
            gate = jax.nn.sigmoid(logit)

            xb = jnp.broadcast_to(x, (32, M))
            x5 = jnp.concatenate([xb[:, 128 * b:128 * (b + 1)] for b in range(5)], axis=0)
            rep = jnp.dot(x5, E, preferred_element_type=F32)
            lhs1 = [jnp.where(diag[:32], rep[32 * b:32 * (b + 1)], 0.0).astype(BF16) for b in range(5)]
            need(AWQ)
            qa = None
            for b in range(5):
                d = jnp.dot(lhs1[b], awq_v[pl.ds(b * 4096, 4096), :], preferred_element_type=F32)
                qa = d if qa is None else qa + d
                tick()
            qa = qa.astype(BF16)

            need(WUK)
            t_diag = []
            for b in range(4):
                t = lax.dot_general(qa, wuk_v[pl.ds(b * 4096, 4096), :], NT, preferred_element_type=F32)
                t_diag.append(jnp.where(diag[:32], t, 0.0).astype(BF16))
                tick()
            qabs4 = lax.dot_general(jnp.concatenate(t_diag, axis=0), E, NT, preferred_element_type=F32)
            qabs = jnp.concatenate([qabs4[32 * b:32 * (b + 1)] for b in range(4)], axis=1).astype(BF16)

            need(CKV)
            s_blocks = []
            for kb in range(4):
                s_blocks.append(lax.dot_general(qabs, ckv_v[pl.ds(kb * 1024, 1024), :], NT,
                                                preferred_element_type=F32))
                tick()
            sa = jnp.concatenate(s_blocks, axis=1) * SCALE
            pa = jnp.exp(sa - jnp.max(sa, axis=-1, keepdims=True))
            la = jnp.sum(pa, axis=-1, keepdims=True)
            pa = pa.astype(BF16)
            tick()
            ca = None
            for kb in range(4):
                d = jnp.dot(pa[:, kb * 1024:(kb + 1) * 1024], ckv_v[pl.ds(kb * 1024, 1024), :],
                            preferred_element_type=F32)
                ca = d if ca is None else ca + d
                tick()
            ca = (ca / la).astype(BF16)

            ca4 = jnp.concatenate([ca[:, 128 * b:128 * (b + 1)] for b in range(4)], axis=0)
            lhs5 = jnp.where(diag, jnp.dot(ca4, E, preferred_element_type=F32), 0.0).astype(BF16)
            need(WUV)
            ctx = None
            for b in range(4):
                d = jnp.dot(lhs5[32 * b:32 * (b + 1)], wuv_v[pl.ds(b * 4096, 4096), :], preferred_element_type=F32)
                ctx = d if ctx is None else ctx + d
                tick()

            ctx_row = jnp.concatenate([jnp.broadcast_to(ctx[h:h + 1, :], (8, 128)) for h in range(H)],
                                      axis=1).astype(BF16)
            need(AWO)
            out_a = None
            for kb in range(4):
                d = jnp.dot(ctx_row[:, kb * 1024:(kb + 1) * 1024], awo_v[pl.ds(kb * 1024, 1024), :],
                            preferred_element_type=F32)
                out_a = d if out_a is None else out_a + d
                tick()

            need(BWQ)
            x8 = jnp.broadcast_to(x, (8, M))
            for kb in range(4):
                qb = jnp.dot(x8, bwq_v[:, pl.ds(kb * 1024, 1024)], preferred_element_type=F32) * SCALE
                for hh in range(8):
                    qb_s[kb * 8 + hh] = qb[:, 128 * hh:128 * (hh + 1)]
                tick()
            need(BWO)
            issue_until(len(stream))
            return gate, out_a

        gate, out_a = pl.run_scoped(prologue, pltpu.SemaphoreType.DMA((9,)))

        tail_pos = [0]

        def issue_tail(count):
            for (n, pos) in tail[tail_pos[0]:tail_pos[0] + count]:
                start_all(kv_copies(n // 2, (n // 2) % NSLOT, n % 2, pos), tail_pos[0] % 2)
                tail_pos[0] += 1

        def issue_rounds(h):
            for j in range(RPH):
                for (n, pos) in _round(AHEAD + j):
                    head = h + n // 2
                    start_all(kv_copies(head, jnp.bitwise_and(head, NSLOT - 1), n % 2, pos), n % 2)

        def scores(h, slot):
            q = qb_s[h].astype(BF16)
            wait_kv(0, slot)
            s = lax.dot_general(q, k_v[slot], NT, preferred_element_type=F32)
            p = jnp.exp(s - jnp.max(s, axis=-1, keepdims=True))
            return p.astype(BF16), jnp.sum(p, axis=-1, keepdims=True)

        def values(h, slot, p, l, acc):
            wait_kv(1, slot)
            o = (jnp.dot(p, v_v[slot], preferred_element_type=F32) / l).astype(BF16)
            row0 = h * DH if isinstance(h, int) else pl.multiple_of(h * DH, DH)
            return acc + jnp.dot(o, bwo_v[pl.ds(row0, DH), :], preferred_element_type=F32)

        def step(h, acc):
            slot = jnp.bitwise_and(h, NSLOT - 1)
            issue_rounds(h)
            p, l = scores(h, slot)
            return values(h, slot, p, l, acc)

        out_b = lax.fori_loop(0, NLOOP, step, jnp.zeros((8, M), F32))
        for h in range(NLOOP, H - 2):
            issue_tail(EPI[h - NLOOP])
            p, l = scores(h, h % NSLOT)
            out_b = values(h, h % NSLOT, p, l, out_b)
        issue_tail(EPI[-2] + EPI[-1])
        p0, l0 = scores(H - 2, (H - 2) % NSLOT)
        p1, l1 = scores(H - 1, (H - 1) % NSLOT)
        out_b = values(H - 2, (H - 2) % NSLOT, p0, l0, out_b)
        out_b = values(H - 1, (H - 1) % NSLOT, p1, l1, out_b)
        return gate * out_a[0:1] + (1.0 - gate) * out_b[0:1]

    mixed = pl.run_scoped(decode, pltpu.SemaphoreType.DMA((2, NSLOT)), pltpu.SemaphoreType.REGULAR((1,)))
    out_ref[...] = mixed.astype(BF16)


@jax.jit
def pallas_gated_mix__compressed_kv_cla__gqa_block_cached__decode_kernel(
    A_x, A_c_kv, A_w_q, A_w_uk, A_w_uv, A_w_o, B_x, B_k_cache, B_v_cache, B_wq, B_wo, gate_w
):
    del B_x
    out = pl.pallas_call(
        _kernel,
        out_shape=jax.ShapeDtypeStruct((1, M), BF16),
        in_specs=[pl.BlockSpec(memory_space=pl.ANY)] * 11,
        out_specs=pl.BlockSpec(memory_space=pltpu.VMEM),
        scratch_shapes=[
            pltpu.VMEM((1, M), BF16),
            pltpu.VMEM((M,), BF16),
            pltpu.VMEM((S, DC), BF16),
            pltpu.VMEM((M * H, DH), BF16),
            pltpu.VMEM((DC * H, DH), BF16),
            pltpu.VMEM((DC * H, DH), BF16),
            pltpu.VMEM((H * DH, M), BF16),
            pltpu.VMEM((M, H * DH), BF16),
            pltpu.VMEM((H * DH, M), BF16),
            pltpu.VMEM((NSLOT, S, DH), BF16),
            pltpu.VMEM((NSLOT, S, DH), BF16),
            pltpu.VMEM((H, 8, DH), F32),
        ],
        compiler_params=pltpu.CompilerParams(vmem_limit_bytes=110 * 1024 * 1024),
    )(
        A_x.reshape(1, M),
        A_c_kv.reshape(S, DC),
        A_w_q.reshape(M * H, DH),
        A_w_uk.reshape(DC * H, DH),
        A_w_uv.reshape(DC * H, DH),
        A_w_o.reshape(H * DH, M),
        B_k_cache.reshape(H, S, DH),
        B_v_cache.reshape(H, S, DH),
        B_wq, B_wo, gate_w)
    return out.reshape(1, 1, M)
```

```python
import jax
import jax.numpy as jnp
from jax import lax
from jax.experimental import pallas as pl
from jax.experimental.pallas import tpu as pltpu

H, DH, M, DC, S = 32, 128, 640, 512, 4096
F32, BF16 = jnp.float32, jnp.bfloat16
NT = (((1,), (1,)), ((), ()))
SCALE = DH ** -0.5

CH = 128
NCH = S // CH
STAG = 4
NACT = NCH // STAG
RPH = 2 * STAG
NSLOT = 8
KV_OFF = 64
AHEAD = 40
LOOK = 72
TICK = 16
EPI = (32, 32, 24, 24, 0)
ROWS640 = (24, 24, 24, 24, 32)

NLOOP = (2 * H * STAG - AHEAD - RPH) // RPH + 1
R_END = RPH * (NLOOP - 1) + AHEAD + RPH


def _linear_pieces(rows, cols):
    out = []
    if cols == H * DH:
        for b in range(rows // 8):
            out += [[(8 * b, 8, 0, 1024), (8 * b, 8, 3072, 1024)], [(8 * b, 8, 1024, 2048)]]
    elif cols == M:
        o = k = 0
        while o < rows:
            r = ROWS640[k % len(ROWS640)]
            out.append([(o, r, 0, cols)])
            o += r
            k += 1
        assert o == rows
    else:
        step = 32 * 1024 // (2 * cols)
        out = [[(o, step, 0, cols)] for o in range(0, rows, step)]
    assert len(out) % NCH == 0
    return out


def _round(r):
    return [(r // STAG - i, r - STAG * (r // STAG - i)) for i in reversed(range(NACT))]


def _queue(item):
    return (item + 1) % 2


def _tail_order():
    order = list(range(2 * H))
    order[-3], order[-2] = order[-2], order[-3]
    out = []
    for n in order:
        first = max(0, R_END - STAG * n)
        if first < NCH:
            c = list(range(first, NCH))
            a, b = c[:len(c) // 2], c[len(c) // 2:]
            for i in range(max(len(a), len(b))):
                if i < len(a):
                    out.append((n, a[i]))
                if i < len(b):
                    out.append((n, b[i]))
    return out


def _kernel(x_hbm, ckv_hbm, awq_hbm, wuk_hbm, wuv_hbm, awo_hbm, k_hbm, v_hbm, bwq_hbm, bwo_hbm, gate_hbm,
            out_ref,
            x_v, gate_v, ckv_v, awq_v, wuk_v, wuv_v, awo_v, bwq_v, bwo_v, k_v, v_v, qb_s):
    AWQ, BWQ, WUK, CKV, WUV, AWO, BWO = range(7)
    weights = [(awq_hbm, awq_v), (bwq_hbm, bwq_v), (wuk_hbm, wuk_v), (ckv_hbm, ckv_v), (wuv_hbm, wuv_v),
               (awo_hbm, awo_v), (bwo_hbm, bwo_v)]
    tail = _tail_order()
    assert len(EPI) == H - NLOOP and sum(EPI) == len(tail)

    def start_all(copies, queue):
        for j, cp in enumerate(copies):
            cp.start(priority=(queue + j) % 2)

    def decode(sem_kv, sem_fence):
        def kv_copies(head, slot, a, pos):
            src, dst = (k_hbm, k_v) if a == 0 else (v_hbm, v_v)
            if pos == 0:
                spans = [(0, KV_OFF), (S - (CH - KV_OFF), CH - KV_OFF)]
            else:
                spans = [(KV_OFF + (pos - 1) * CH, CH)]
            return [pltpu.make_async_copy(src.at[head, pl.ds(o, n)], dst.at[slot, pl.ds(o, n)], sem_kv.at[a, slot])
                    for (o, n) in spans]

        def wait_kv(a, slot):
            d = (k_v if a == 0 else v_v).at[slot]
            pltpu.make_async_copy(d, d, sem_kv.at[a, slot]).wait()

        def prologue(sem_w):
            def w_copies(i, piece):
                src, dst = weights[i]
                return [pltpu.make_async_copy(src.at[pl.ds(r0, nr), pl.ds(c0, nc)],
                                              dst.at[pl.ds(r0, nr), pl.ds(c0, nc)], sem_w.at[i])
                        for (r0, nr, c0, nc) in piece]

            w_items = []
            for i, (_, dst) in enumerate(weights):
                pieces = _linear_pieces(*dst.shape)
                w_items += [(i, pieces[j:j + NCH]) for j in range(0, len(pieces), NCH)]
            n_w = len(w_items)
            stream, last_piece, issued = [], {}, [0]
            for r in range(STAG * n_w + AHEAD):
                for (g, pos) in _round(r):
                    if g < 0:
                        continue
                    if g < n_w:
                        i, pieces = w_items[g]
                        stream.append(lambda i=i, p=pieces[pos], q=_queue(g): start_all(w_copies(i, p), q))
                        last_piece[i] = len(stream)
                    else:
                        n = g - n_w
                        stream.append(lambda n=n, pos=pos, q=_queue(g):
                                      start_all(kv_copies(n // 2, (n // 2) % NSLOT, n % 2, pos), q))

            def issue_until(n):
                n = min(n, len(stream))
                while issued[0] < n:
                    stream[issued[0]]()
                    issued[0] += 1

            def need(i):
                issue_until(last_piece[i] + LOOK)
                d = weights[i][1]
                pltpu.make_async_copy(d, d, sem_w.at[i]).wait()

            def tick():
                pl.semaphore_signal(sem_fence.at[0], 1)
                pl.semaphore_wait(sem_fence.at[0], 1)
                issue_until(issued[0] + TICK)

            x_cp = pltpu.make_async_copy(x_hbm, x_v, sem_w.at[7])
            g_cp = pltpu.make_async_copy(gate_hbm, gate_v, sem_w.at[8])
            x_cp.start()
            g_cp.start()
            issue_until(LOOK)

            lane = lax.broadcasted_iota(jnp.int32, (128, 4096), 1)
            row = lax.broadcasted_iota(jnp.int32, (128, 4096), 0)
            E = jnp.where((lane >> 5) == row, 1.0, 0.0).astype(BF16)
            diag = (lane & 31) == (row & 31)

            x_cp.wait()
            g_cp.wait()
            x = x_v[...]
            logit = jnp.sum(x.astype(F32) * gate_v[...].reshape(1, M).astype(F32), axis=-1, keepdims=True)
            gate = jax.nn.sigmoid(logit)

            xb = jnp.broadcast_to(x, (32, M))
            x5 = jnp.concatenate([xb[:, 128 * b:128 * (b + 1)] for b in range(5)], axis=0)
            rep = jnp.dot(x5, E, preferred_element_type=F32)
            lhs1 = [jnp.where(diag[:32], rep[32 * b:32 * (b + 1)], 0.0).astype(BF16) for b in range(5)]
            need(AWQ)
            qa = None
            for b in range(5):
                d = jnp.dot(lhs1[b], awq_v[pl.ds(b * 4096, 4096), :], preferred_element_type=F32)
                qa = d if qa is None else qa + d
                tick()
            qa = qa.astype(BF16)

            need(WUK)
            t_diag = []
            for b in range(4):
                t = lax.dot_general(qa, wuk_v[pl.ds(b * 4096, 4096), :], NT, preferred_element_type=F32)
                t_diag.append(jnp.where(diag[:32], t, 0.0).astype(BF16))
                tick()
            qabs4 = lax.dot_general(jnp.concatenate(t_diag, axis=0), E, NT, preferred_element_type=F32)
            qabs = jnp.concatenate([qabs4[32 * b:32 * (b + 1)] for b in range(4)], axis=1).astype(BF16)

            need(CKV)
            s_blocks = []
            for kb in range(4):
                s_blocks.append(lax.dot_general(qabs, ckv_v[pl.ds(kb * 1024, 1024), :], NT,
                                                preferred_element_type=F32))
                tick()
            sa = jnp.concatenate(s_blocks, axis=1) * SCALE
            pa = jnp.exp(sa - jnp.max(sa, axis=-1, keepdims=True))
            la = jnp.sum(pa, axis=-1, keepdims=True)
            pa = pa.astype(BF16)
            tick()
            ca = None
            for kb in range(4):
                d = jnp.dot(pa[:, kb * 1024:(kb + 1) * 1024], ckv_v[pl.ds(kb * 1024, 1024), :],
                            preferred_element_type=F32)
                ca = d if ca is None else ca + d
                tick()
            ca = (ca / la).astype(BF16)

            ca4 = jnp.concatenate([ca[:, 128 * b:128 * (b + 1)] for b in range(4)], axis=0)
            lhs5 = jnp.where(diag, jnp.dot(ca4, E, preferred_element_type=F32), 0.0).astype(BF16)
            need(WUV)
            ctx = None
            for b in range(4):
                d = jnp.dot(lhs5[32 * b:32 * (b + 1)], wuv_v[pl.ds(b * 4096, 4096), :], preferred_element_type=F32)
                ctx = d if ctx is None else ctx + d
                tick()

            ctx_row = jnp.concatenate([jnp.broadcast_to(ctx[h:h + 1, :], (8, 128)) for h in range(H)],
                                      axis=1).astype(BF16)
            need(AWO)
            out_a = None
            for kb in range(4):
                d = jnp.dot(ctx_row[:, kb * 1024:(kb + 1) * 1024], awo_v[pl.ds(kb * 1024, 1024), :],
                            preferred_element_type=F32)
                out_a = d if out_a is None else out_a + d
                tick()

            need(BWQ)
            x8 = jnp.broadcast_to(x, (8, M))
            for kb in range(4):
                qb = jnp.dot(x8, bwq_v[:, pl.ds(kb * 1024, 1024)], preferred_element_type=F32) * SCALE
                for hh in range(8):
                    qb_s[kb * 8 + hh] = qb[:, 128 * hh:128 * (hh + 1)]
                tick()
            need(BWO)
            issue_until(len(stream))
            return gate, out_a

        gate, out_a = pl.run_scoped(prologue, pltpu.SemaphoreType.DMA((9,)))

        tail_pos = [0]

        def issue_tail(count):
            for (n, pos) in tail[tail_pos[0]:tail_pos[0] + count]:
                start_all(kv_copies(n // 2, (n // 2) % NSLOT, n % 2, pos), tail_pos[0] % 2)
                tail_pos[0] += 1

        def issue_rounds(h):
            for j in range(RPH):
                for (n, pos) in _round(AHEAD + j):
                    head = h + n // 2
                    start_all(kv_copies(head, jnp.bitwise_and(head, NSLOT - 1), n % 2, pos), _queue(n))

        def scores(h, slot):
            q = qb_s[h].astype(BF16)
            wait_kv(0, slot)
            s = lax.dot_general(q, k_v[slot], NT, preferred_element_type=F32)
            p = jnp.exp(s - jnp.max(s, axis=-1, keepdims=True))
            return p.astype(BF16), jnp.sum(p, axis=-1, keepdims=True)

        def values(h, slot, p, l, acc):
            wait_kv(1, slot)
            o = (jnp.dot(p, v_v[slot], preferred_element_type=F32) / l).astype(BF16)
            row0 = h * DH if isinstance(h, int) else pl.multiple_of(h * DH, DH)
            return acc + jnp.dot(o, bwo_v[pl.ds(row0, DH), :], preferred_element_type=F32)

        def step(h, acc):
            slot = jnp.bitwise_and(h, NSLOT - 1)
            issue_rounds(h)
            p, l = scores(h, slot)
            return values(h, slot, p, l, acc)

        out_b = lax.fori_loop(0, NLOOP, step, jnp.zeros((8, M), F32))
        for h in range(NLOOP, H - 2):
            issue_tail(EPI[h - NLOOP])
            p, l = scores(h, h % NSLOT)
            out_b = values(h, h % NSLOT, p, l, out_b)
        issue_tail(EPI[-2] + EPI[-1])
        p0, l0 = scores(H - 2, (H - 2) % NSLOT)
        p1, l1 = scores(H - 1, (H - 1) % NSLOT)
        out_b = values(H - 2, (H - 2) % NSLOT, p0, l0, out_b)
        out_b = values(H - 1, (H - 1) % NSLOT, p1, l1, out_b)
        return gate * out_a[0:1] + (1.0 - gate) * out_b[0:1]

    mixed = pl.run_scoped(decode, pltpu.SemaphoreType.DMA((2, NSLOT)), pltpu.SemaphoreType.REGULAR((1,)))
    out_ref[...] = mixed.astype(BF16)


@jax.jit
def pallas_gated_mix__compressed_kv_cla__gqa_block_cached__decode_kernel(
    A_x, A_c_kv, A_w_q, A_w_uk, A_w_uv, A_w_o, B_x, B_k_cache, B_v_cache, B_wq, B_wo, gate_w
):
    del B_x
    out = pl.pallas_call(
        _kernel,
        out_shape=jax.ShapeDtypeStruct((1, M), BF16),
        in_specs=[pl.BlockSpec(memory_space=pl.ANY)] * 11,
        out_specs=pl.BlockSpec(memory_space=pltpu.VMEM),
        scratch_shapes=[
            pltpu.VMEM((1, M), BF16),
            pltpu.VMEM((M,), BF16),
            pltpu.VMEM((S, DC), BF16),
            pltpu.VMEM((M * H, DH), BF16),
            pltpu.VMEM((DC * H, DH), BF16),
            pltpu.VMEM((DC * H, DH), BF16),
            pltpu.VMEM((H * DH, M), BF16),
            pltpu.VMEM((M, H * DH), BF16),
            pltpu.VMEM((H * DH, M), BF16),
            pltpu.VMEM((NSLOT, S, DH), BF16),
            pltpu.VMEM((NSLOT, S, DH), BF16),
            pltpu.VMEM((H, 8, DH), F32),
        ],
        compiler_params=pltpu.CompilerParams(vmem_limit_bytes=110 * 1024 * 1024),
    )(
        A_x.reshape(1, M),
        A_c_kv.reshape(S, DC),
        A_w_q.reshape(M * H, DH),
        A_w_uk.reshape(DC * H, DH),
        A_w_uv.reshape(DC * H, DH),
        A_w_o.reshape(H * DH, M),
        B_k_cache.reshape(H, S, DH),
        B_v_cache.reshape(H, S, DH),
        B_wq, B_wo, gate_w)
    return out.reshape(1, 1, M)
```
